```python
import os as _os
_os.environ.setdefault("JAX_PLATFORMS", "cpu")
import jax
import jax.numpy as jnp

def _softmax(x, axis=-1):
    return jax.nn.softmax(x, axis=axis)
def _gelu(x):
    return jax.nn.gelu(x, approximate=True)
def _silu(x):
    return jax.nn.silu(x)
def _sigmoid(x):
    return jax.nn.sigmoid(x)
def _layernorm(x, axis=-1, eps=1e-5):
    m = jnp.mean(x, axis=axis, keepdims=True)
    v = jnp.var(x, axis=axis, keepdims=True)
    return (x - m) / jnp.sqrt(v + eps)
def _scatter_add(tgt, idx, src, axis=0):
    return tgt.at[idx].add(src)
def _segment_sum(src, seg, n):
    return jax.ops.segment_sum(src, seg, n)
class _Rng:
    def __init__(self, key):
        self._k = key
    def _next(self):
        self._k, sub = jax.random.split(self._k)
        return sub
    def normal(self, shape):
        return jax.random.normal(self._next(), shape, dtype=jnp.bfloat16)
    def randint(self, lo, hi, shape):
        return jax.random.randint(self._next(), shape, lo, hi, dtype=jnp.int32)
    def uniform(self, shape, lo=0.0, hi=1.0):
        return jax.random.uniform(self._next(), shape, jnp.bfloat16, lo, hi)
    def permutation(self, n):
        return jax.random.permutation(self._next(), n)


kernel_name = 'concat_heads__sliding_block__ssm_conv_s4__prompt'

def setup_inputs():
    _rng = _Rng(jax.random.key(int.from_bytes(__import__("os").urandom(4), "little")))
    _w = (lambda a: (lambda t: t.astype(jnp.bfloat16) if jnp.issubdtype(t.dtype, jnp.floating) else t)(jnp.asarray(a)))
    def _A_setup():
        B, S, D = 1, 2048, 512
        return {
            "x": _w((lambda *s: _rng.normal(s) * 0.2)(B, S, D)),
            "wqkv": _w((lambda *s: _rng.normal(s) * 0.2)(D, 3 * D)),
            "wo": _w((lambda *s: _rng.normal(s) * 0.05)(D, D)),
        }
    _A_in = _A_setup()

    def _B_setup():
        B, L, D, N = 1, 2048, 512, 128
        A_re = -jnp.exp((lambda *s: _rng.normal(s) * 0.8)(D, N))
        A_im = jnp.pi * (lambda *s: _rng.normal(s) * 0.8)(D, N)
        B_re = (lambda *s: _rng.normal(s) * 0.8)(D, N)
        B_im = (lambda *s: _rng.normal(s) * 0.8)(D, N)
        C_re = (lambda *s: _rng.normal(s) * 0.8)(D, N)
        C_im = (lambda *s: _rng.normal(s) * 0.8)(D, N)
        log_dt = (lambda *s: _rng.normal(s) * 0.8)(D) * 0.5 - 4.0
        Dskip = (lambda *s: _rng.normal(s) * 0.05)(D)
        return {
            "u": _w((lambda *s: _rng.normal(s) * 0.05)(B, L, D)),
            "A_re": _w(A_re),
            "A_im": _w(A_im),
            "B_re": _w(B_re),
            "B_im": _w(B_im),
            "C_re": _w(C_re),
            "C_im": _w(C_im),
            "log_dt": _w(log_dt),
            "Dskip": _w(Dskip),
        }
    _B_in = _B_setup()

    return {
        "A_x": _A_in["x"],
        "A_wqkv": _A_in["wqkv"],
        "A_wo": _A_in["wo"],
        "B_u": _B_in["u"],
        "B_A_re": _B_in["A_re"],
        "B_A_im": _B_in["A_im"],
        "B_B_re": _B_in["B_re"],
        "B_B_im": _B_in["B_im"],
        "B_C_re": _B_in["C_re"],
        "B_C_im": _B_in["C_im"],
        "B_log_dt": _B_in["log_dt"],
        "B_Dskip": _B_in["Dskip"],
    }

def reference(A_x, A_wqkv, A_wo, B_u, B_A_re, B_A_im, B_B_re, B_B_im, B_C_re, B_C_im, B_log_dt, B_Dskip):
    def _A_ref(x, wqkv, wo):
        B, S, D = x.shape
        H = 32; Dh = D // H; W = 256
        qkv = (lambda x, *d: x.transpose(*d))((x @ wqkv).reshape(B, S, 3, H, Dh), 2, 0, 3, 1, 4)
        q, k, v = qkv[0], qkv[1], qkv[2]
        scores = jnp.einsum("bhqd,bhkd->bhqk", q, k) * (Dh ** -0.5)
        idx = jnp.arange(S)
        mask = (idx[:, None] - idx[None, :] >= 0) & (idx[:, None] - idx[None, :] < W)
        scores = jnp.where(mask[None, None], scores, -1e9)
        p = _softmax(scores, axis=-1)
        o = jnp.einsum("bhqk,bhkd->bhqd", p, v)
        return (lambda x, *d: x.transpose(*d))(o, 0, 2, 1, 3).reshape(B, S, D) @ wo

    def _B_ref(u, A_re, A_im, B_re, B_im, C_re, C_im, log_dt, Dskip):
        Bsz, L, D = u.shape
        dt = jnp.exp(log_dt)[:, None]
        A = A_re + 1j * A_im
        Bc = B_re + 1j * B_im
        Cc = C_re + 1j * C_im
        logdA = dt * A
        dB = dt * Bc
        l = (lambda x, dt: x.astype(dt))(jnp.arange(L), A_re.dtype)
        P = jnp.exp(logdA[:, :, None] * l[None, None, :])
        K = jnp.einsum("dn,dnl,dn->dl", Cc, P, dB).real
        L2 = 2 * L
        Kp = jnp.pad(K, ((0, 0), (0, L)))
        up = (lambda x, *d: x.transpose(*d))(u, 0, 2, 1)
        up = jnp.pad(up, ((0, 0), (0, 0), (0, L)))
        Kf = (lambda x, axes=(-2,-1): jnp.fft.rfft2(x.astype(jnp.float32), axes=axes))(Kp[:, None, :], axes=(-2, -1))
        Uf = (lambda x, axes=(-2,-1): jnp.fft.rfft2(x.astype(jnp.float32), axes=axes))(up[:, :, None, :], axes=(-2, -1))
        Yf = Uf * Kf[None, :, :, :]
        y = (lambda x, s, axes=(-2,-1): jnp.fft.irfft2(x, s=s, axes=axes).astype(jnp.bfloat16))(Yf, (1, L2), axes=(-2, -1))[:, :, 0, :L]
        y = (lambda x, *d: x.transpose(*d))(y, 0, 2, 1) + u * Dskip[None, None, :]
        return y

    a = _A_ref(A_x, A_wqkv, A_wo)
    b = _B_ref(B_u, B_A_re, B_A_im, B_B_re, B_B_im, B_C_re, B_C_im, B_log_dt, B_Dskip)
    return jnp.concatenate([a, b], axis=-1)
```

```python
import functools, math
import jax, jax.numpy as jnp, numpy as np
from jax import lax
from jax.experimental import pallas as pl
from jax.experimental.pallas import tpu as pltpu

f32, bf16, i32 = jnp.float32, jnp.bfloat16, jnp.int32
S, D = 2048, 512
QSCALE = 0.25 * math.log2(math.e)
NEG = -1e30
T = 64
NC = S // T
PR = 33
YR = 40
SR = 9
NT = (((1,), (1,)), ((), ()))
DO_A = 1; DO_B = 1

def iota(shape, dim):
    return lax.broadcasted_iota(jnp.int32, shape, dim)
def pack(x):
    return pltpu.bitcast(x, i32)
def unpack(x):
    return pltpu.bitcast(x, bf16)
def mo(x, m):
    return x if isinstance(x, int) else pl.multiple_of(x, m)
def cmul(ar, ai, br, bi):
    return ar * br - ai * bi, ar * bi + ai * br

def proj_block(i, x_ref, wqkv_ref, qc_s, k_s, vt_s):
    R = 256
    r0 = mo(i * R, R)
    rp = mo(i * (R // 2), R // 2)
    xb = x_ref[pl.ds(r0, R), :]
    q = jnp.dot(xb, wqkv_ref[:, 0:512], preferred_element_type=f32) * QSCALE
    oddh = ((iota((64, 128), 1) // 16) % 2) == 1
    for j in range(2):
        lo, hi = q[j * 128:j * 128 + 64], q[j * 128 + 64:j * 128 + 128]
        for hg in range(4):
            a, b = lo[:, hg * 128:(hg + 1) * 128], hi[:, hg * 128:(hg + 1) * 128]
            m = jnp.concatenate([jnp.where(oddh, b, a), jnp.where(oddh, a, b)], 0).astype(bf16)
            qc_s[2 * i + j, pl.ds(hg * 64, 64), :] = pack(m.T)
    k = jnp.dot(xb, wqkv_ref[:, 512:1024], preferred_element_type=f32).astype(bf16)
    for hg in range(4):
        k_s[hg, pl.ds(rp, R // 2), :] = pack(k[:, hg * 128:(hg + 1) * 128])
    v = jnp.dot(xb, wqkv_ref[:, 1024:1536], preferred_element_type=f32).astype(bf16)
    for j in range(2):
        vt_s[2 * i + j] = pack(v[j * 128:(j + 1) * 128, :].T)

def win(qb, odd, static_edge):
    if static_edge:
        b = 2 * qb + (1 if odd else 0)
        rmin = max(0, 256 - 64 * b)
        return rmin, 64 * b - 256 + rmin
    return 0, qb * 128 - 256 + (64 if odd else 0)

def qk_stage(qb, gi, static_edge, qc_s, k_s, st):
    hg = gi // 2
    lo = iota((8, 128), 1) < 64
    zero = jnp.zeros((8, 128), i32)
    t = 0
    for hp in (2 * gi, 2 * gi + 1):
        h1, h2 = 2 * hp, 2 * hp + 1
        q1 = qc_s[qb, pl.ds(h1 * 8, 8), :]
        q2 = qc_s[qb, pl.ds(h2 * 8, 8), :]
        for odd in (False, True):
            blocks = [zero] * 8
            blocks[h1 % 8] = jnp.where(lo, zero, q1) if odd else jnp.where(lo, q1, zero)
            blocks[h2 % 8] = jnp.where(lo, q2, zero) if odd else jnp.where(lo, zero, q2)
            w = unpack(jnp.concatenate(blocks, 0))
            rmin, key0 = win(qb, odd, static_edge)
            n = 320 - rmin
            kk = k_s[hg, pl.ds(mo(key0 // 2, 32), n // 2), :]
            st[t, pl.ds(rmin, n), :] = jnp.dot(unpack(kk), w, preferred_element_type=f32)
            t += 1

def smpv_stage(qb, gi, static_edge, st, vt_s, ot_s):
    mask = iota((64, 128), 0) > (iota((64, 128), 1) % 64)
    zero = jnp.zeros((64, 128), f32)
    t = 0
    take_e = (iota((32, 128), 1) < 64) == (iota((32, 128), 0) < 16)
    for hp in (2 * gi, 2 * gi + 1):
        zs = []
        for odd in (False, True):
            rmin, _ = win(qb, odd, static_edge)
            bot = st[t, 256:320, :]
            has_top = rmin == 0
            comb = jnp.where(mask, st[t, 0:64, :], bot) if has_top else jnp.where(mask, NEG, bot)
            m = jnp.max(comb, axis=0, keepdims=True)
            m0 = max(rmin, 64)
            nm = 256 - m0
            if nm:
                mid = st[t, pl.ds(m0, nm), :]
                m = jnp.maximum(m, jnp.max(mid, axis=0, keepdims=True))
            pc = jnp.exp2(comb - m)
            l = jnp.sum(pc, axis=0, keepdims=True)
            if nm:
                pm = jnp.exp2(mid - m)
                l = l + jnp.sum(pm, axis=0, keepdims=True)
            pbot = jnp.where(mask, 0.0, pc)
            ptop = jnp.where(mask, pc, 0.0) if has_top else None
            pieces = [None] * 5
            pieces[4] = pbot
            if has_top:
                pieces[0] = ptop
            for k in range(m0 // 64, 4):
                pieces[k] = pm[k * 64 - m0:(k + 1) * 64 - m0]
            sl = [(-1, 0), (1, 2), (3, 4)] if odd else [(0, 1), (2, 3), (4, -1)]
            z = None
            for ci in range(3):
                a = pieces[sl[ci][0]] if sl[ci][0] >= 0 else None
                b = pieces[sl[ci][1]] if sl[ci][1] >= 0 else None
                if a is None and b is None:
                    continue
                ch = jnp.concatenate([zero if a is None else a, zero if b is None else b], 0).astype(bf16)
                vt = unpack(vt_s[qb - 2 + ci, pl.ds(hp * 16, 16), :])
                d = jnp.dot(vt, ch, preferred_element_type=f32)
                z = d if z is None else z + d
            zs.append(z * (1.0 / l))
            t += 1
        o = jnp.where(take_e, zs[0], zs[1]).astype(bf16)
        ot_s[qb, pl.ds(hp * 16, 16), :] = pack(o)

def oproj_tr(qb, ot_s, o_s):
    oddh = ((iota((32, 128), 1) // 16) % 2) == 1
    for g in range(4):
        tp = pack(unpack(ot_s[qb, pl.ds(g * 64, 64), :]).T)
        a, b = tp[0:32], tp[32:64]
        o_s[g] = jnp.concatenate([jnp.where(oddh, b, a), jnp.where(oddh, a, b)], 0)

def oproj_mm(qb, n, o_s, wo_ref, out_ref):
    acc = None
    for g in range(4):
        d = jnp.dot(unpack(o_s[g]), wo_ref[pl.ds(g * 128, 128), pl.ds(n * 128, 128)], preferred_element_type=f32)
        acc = d if acc is None else acc + d
    out_ref[pl.ds(mo(qb * 128, 128), 128), pl.ds(n * 128, 128)] = acc.astype(bf16)

def b_prep(blk, dtc_s, are, aim, bre, bim, cre, cim, base_s, l8_s, lt_s, rt_s, wre_s):
    r0 = mo(blk * 32, 32)
    rows = pl.ds(r0, 32)
    dtc = dtc_s[rows, :]
    zr = dtc * are[rows, :].astype(f32)
    zi = dtc * aim[rows, :].astype(f32)
    mag = jnp.exp(zr)
    lr, li = mag * jnp.cos(zi), mag * jnp.sin(zi)
    wr, wi = cmul(cre[rows, :].astype(f32), cim[rows, :].astype(f32), dtc * bre[rows, :].astype(f32), dtc * bim[rows, :].astype(f32))
    wre_s[rows, :] = wr
    a, b = cmul(wr, wi, lr, li)
    m = jnp.sqrt(a * a + b * b)
    t = jnp.sqrt(0.5 * (m + jnp.abs(a)))
    ts = jnp.where(t > 0.0, t, 1.0)
    o = jnp.where(t > 0.0, 0.5 * b / ts, 0.0)
    pos = a >= 0.0
    rr = jnp.where(pos, t, jnp.abs(o))
    ri = jnp.where(pos, o, jnp.where(b >= 0.0, t, -t))
    rt_s[0, rows, :] = rr
    rt_s[1, rows, :] = ri
    pr, pi = rr, ri
    for s in range(8):
        base_s[0, pl.ds(r0 * 8 + s, 32, stride=8), :] = pr
        base_s[1, pl.ds(r0 * 8 + s, 32, stride=8), :] = pi
        if s < 7:
            pr, pi = cmul(pr, pi, lr, li)
    qr, qi = lr, li
    for k in range(6):
        qr, qi = qr * qr - qi * qi, 2.0 * qr * qi
        if k == 2:
            l8_s[0, rows, :] = qr
            l8_s[1, rows, :] = qi
    lt_s[0, rows, :] = qr
    lt_s[1, rows, :] = qi

def u_prep(tp, c, u_ref, ur_s):
    r0 = mo(c * T, T)
    rev = 7 - iota((8, 128), 0)
    parts = []
    for j in range(2):
        v = u_ref[pl.ds(r0, T), pl.ds((2 * tp + j) * 128, 128)].astype(f32)
        parts += [jnp.take_along_axis(v[8 * (7 - k):8 * (8 - k), :], rev, axis=0) for k in range(8)]
    mt = jnp.concatenate(parts, axis=0).T
    ur_s[pl.ds(tp * 128 * PR + c, 128, stride=PR), :] = mt

def gen_p(d, base_s, l8_s):
    r8 = mo(d * 8, 8)
    pr, pi = base_s[0, pl.ds(r8, 8), :], base_s[1, pl.ds(r8, 8), :]
    mr = jnp.broadcast_to(l8_s[0, pl.ds(d, 1), :], (8, 128))
    mi = jnp.broadcast_to(l8_s[1, pl.ds(d, 1), :], (8, 128))
    rs, is_ = [pr], [pi]
    for v in range(7):
        pr, pi = cmul(pr, pi, mr, mi)
        rs.append(pr); is_.append(pi)
    return jnp.concatenate(rs, 0), jnp.concatenate(is_, 0)

class BGroup:
    def __init__(self, gi, sb, R):
        self.tp = gi // 16
        self.p0 = (gi % 16) * 8
        self.d0 = self.tp * 256 + self.p0
        self.sb = sb; self.R = R
        self.Ws = [None] * 8
        self.h = [None, None]
    def xrows(self, i):
        return self.R["ur_s"][pl.ds((self.tp * 128 + self.p0 + i) * PR, NC), :]
    def stage_a(self, i):
        R, sb = self.R, self.sb
        lo = iota((NC, 128), 1) < T
        w = [gen_p(self.d0 + i + 128 * j, R["base_s"], R["l8_s"]) for j in range(2)]
        wre = jnp.concatenate([w[0][0], w[1][0]], 0).astype(bf16)
        wim = jnp.concatenate([w[0][1], w[1][1]], 0).astype(bf16)
        x = self.xrows(i)
        lhs = jnp.concatenate([jnp.where(lo, x, 0.0), jnp.where(lo, 0.0, x)], 0).astype(bf16)
        sre = jnp.dot(lhs, wre, preferred_element_type=f32)
        sim = jnp.dot(lhs, wim, preferred_element_type=f32)
        for j in range(2):
            sb[j, 0, pl.ds(i, NC, stride=SR), :] = sre[j * NC:(j + 1) * NC]
            sb[j, 1, pl.ds(i, NC, stride=SR), :] = sim[j * NC:(j + 1) * NC]
        self.Ws[i] = (wre, wim)
    def stage_r(self, c0, c1):
        R, sb = self.R, self.sb
        for j in range(2):
            rows = pl.ds(mo(self.d0 + 128 * j, 8), 8)
            ar, ai = R["lt_s"][0, rows, :], R["lt_s"][1, rows, :]
            if c0 == 0:
                hr = sb[j, 0, pl.ds(0, 8), :]
                hi = sb[j, 1, pl.ds(0, 8), :]
                sb[j, 0, pl.ds(0, 8), :] = R["rt_s"][0, rows, :]
                sb[j, 1, pl.ds(0, 8), :] = -R["rt_s"][1, rows, :]
            else:
                hr, hi = self.h[j]
            for c in range(max(c0, 1), c1):
                sr = sb[j, 0, pl.ds(c * SR, 8), :]
                si = sb[j, 1, pl.ds(c * SR, 8), :]
                sb[j, 0, pl.ds(c * SR, 8), :] = hr
                sb[j, 1, pl.ds(c * SR, 8), :] = -hi
                if c < NC - 1:
                    hr, hi = ar * hr - ai * hi + sr, ar * hi + ai * hr + si
            self.h[j] = (hr, hi)
    def stage_c(self, i):
        R, sb = self.R, self.sb
        lo = iota((NC, 128), 1) < T
        lane = iota((8, 128), 1)
        rev = 7 - iota((8, 128), 0)
        row0 = iota((NC, 128), 0) == 0
        wre, wim = self.Ws[i]
        gre = jnp.concatenate([sb[j, 0, pl.ds(i, NC, stride=SR), :] for j in range(2)], 0).astype(bf16)
        gim = jnp.concatenate([sb[j, 1, pl.ds(i, NC, stride=SR), :] for j in range(2)], 0).astype(bf16)
        y = lax.dot_general(gre, wre, NT, preferred_element_type=f32) + lax.dot_general(gim, wim, NT, preferred_element_type=f32)
        yi = jnp.where(lo, y[0:NC], y[NC:2 * NC])
        kc = jnp.broadcast_to(yi[0:1, :], (8, 128))
        h0, h1 = [], []
        for v in range(8):
            r = pltpu.roll(kc, 57 - 8 * v, 1, stride=1, stride_axis=0)
            r = jnp.take_along_axis(r, rev, axis=0)
            sg = lane + iota((8, 128), 0) + 8 * v
            h0.append(jnp.where((lane < 64) & (sg >= 64), r, 0.0))
            h1.append(jnp.where(sg >= 128, r, 0.0))
        hk = jnp.concatenate(h0 + h1, 0).astype(bf16)
        yy = jnp.where(row0, 0.0, yi) + jnp.dot(self.xrows(i).astype(bf16), hk, preferred_element_type=f32)
        R["yb_s"][pl.ds(mo((self.tp * 128 + self.p0 + i) * YR, 8), NC), :] = yy

def b_out(q, u_ref, yb_s, coef_s, out_ref):
    tp = q // NC; c = q % NC
    mt = yb_s[pl.ds(tp * 128 * YR + c, 128, stride=YR), :].T
    r0 = mo(c * T, T)
    for j in range(2):
        lt = 2 * tp + j
        cf = coef_s[lt]
        uu = u_ref[pl.ds(r0, T), pl.ds(mo(lt * 128, 128), 128)].astype(f32)
        out_ref[pl.ds(r0, T), pl.ds(mo(D + lt * 128, 128), 128)] = (mt[j * T:(j + 1) * T] + uu * jnp.concatenate([cf] * 8, 0)).astype(bf16)

NBG = 4
SCHED = 0

def kernel(x_ref, wqkv_ref, wo_ref, u_ref, are, aim, bre, bim, cre, cim, ldt_ref, dsk_ref, out_ref,
           qc_s, k_s, vt_s, ot_s, o_s, st0, st1,
           ur_s, base_s, l8_s, lt_s, rt_s, wre_s, sb0, sb1, yb_s, coef_s, dtc_s):
    R = dict(ur_s=ur_s, base_s=base_s, l8_s=l8_s, lt_s=lt_s, rt_s=rt_s, yb_s=yb_s)
    if DO_B:
        for g in range(4):
            dt = jnp.exp(ldt_ref[g:g + 1, :].astype(f32)).astype(bf16).astype(f32)
            dtc_s[g * 128:(g + 1) * 128, :] = jnp.broadcast_to(dt, (128, 128)).T
    def phase1(i, c):
        if DO_B:
            for k in range(2):
                b_prep(2 * i + k, dtc_s, are, aim, bre, bim, cre, cim, base_s, l8_s, lt_s, rt_s, wre_s)
            for k in range(8):
                q = i * 8 + k
                u_prep(q // NC, q % NC, u_ref, ur_s)
        if DO_A:
            proj_block(i, x_ref, wqkv_ref, qc_s, k_s, vt_s)
        return c
    lax.fori_loop(0, 8, phase1, 0)
    if DO_B:
        ones = jnp.ones((8, 128), f32)
        for g in range(4):
            k0 = lax.dot_general(ones, wre_s[g * 128:(g + 1) * 128, :], NT, preferred_element_type=f32, precision=lax.Precision.HIGHEST)
            coef_s[g] = k0 + jnp.broadcast_to(dsk_ref[g:g + 1, :].astype(f32), (8, 128))

    bufs = [st0, st1]
    def body(qb, edge, next_edge, kind, first=False, last=False):
        bg = [[] for _ in range(8)]
        if DO_A and not first:
            bg[0].append(lambda: oproj_tr(qb - 1, ot_s, o_s))
            for n in range(4):
                bg[1 + n].append(functools.partial(oproj_mm, qb - 1, n, o_s, wo_ref, out_ref))
        if DO_B and kind == 'X':
            G = [BGroup(qb * NBG + k, [sb0, sb1][k % 2], R) for k in range(NBG)]
            steps = []
            for k, g in enumerate(G):
                steps += [(k * 2 + 0, functools.partial(g.stage_a, i)) for i in range(8)]
                steps += [(k * 2 + 1, functools.partial(g.stage_r, 0, NC))]
                steps += [(k * 2 + 2, functools.partial(g.stage_c, i)) for i in range(8)]
            nt = NBG * 2 + 1
            for tm, fn in sorted(steps, key=lambda s: s[0]):
                bg[min(7, tm * 8 // nt)].append(fn)
        if DO_B and kind == 'Y':
            for k in range(8):
                bg[k].append(functools.partial(b_out, (qb - 8) * 8 + k, u_ref, yb_s, coef_s, out_ref))
        for u in range(8):
            if DO_A:
                if u < 7:
                    qk_stage(qb, u + 1, edge, qc_s, k_s, bufs[(u + 1) % 2])
                elif not last:
                    qk_stage(qb + 1, 0, next_edge, qc_s, k_s, bufs[(u + 1) % 2])
            if SCHED == 0:
                for fn in bg[u]: fn()
            if DO_A:
                smpv_stage(qb, u, edge, bufs[u % 2], vt_s, ot_s)
            if SCHED == 1:
                for fn in bg[u]: fn()

    if DO_A:
        qk_stage(0, 0, True, qc_s, k_s, st0)
    body(0, True, True, 'X', first=True)
    body(1, True, False, 'X')
    def loopX(qb, c):
        body(qb, False, False, 'X'); return c
    lax.fori_loop(2, 8, loopX, 0)
    def loopY(qb, c):
        body(qb, False, False, 'Y'); return c
    lax.fori_loop(8, 15, loopY, 0)
    body(15, False, False, 'Y', last=True)
    if DO_A:
        oproj_tr(15, ot_s, o_s)
        for n in range(4):
            oproj_mm(15, n, o_s, wo_ref, out_ref)
    if not DO_B:
        out_ref[:, D:] = jnp.zeros((S, D), bf16)
    if not DO_A:
        out_ref[:, :D] = jnp.zeros((S, D), bf16)

SCRATCH = [
    pltpu.VMEM((16, 256, 128), i32),
    pltpu.VMEM((4, S // 2, 128), i32),
    pltpu.VMEM((16, 256, 128), i32),
    pltpu.VMEM((16, 256, 128), i32),
    pltpu.VMEM((4, 64, 128), i32),
    pltpu.VMEM((4, 320, 128), f32), pltpu.VMEM((4, 320, 128), f32),
    pltpu.VMEM((256 * PR, 128), f32),
    pltpu.VMEM((2, D * 8, 128), f32),
    pltpu.VMEM((2, D, 128), f32), pltpu.VMEM((2, D, 128), f32), pltpu.VMEM((2, D, 128), f32),
    pltpu.VMEM((D, 128), f32),
    pltpu.VMEM((2, 2, NC * SR, 128), f32), pltpu.VMEM((2, 2, NC * SR, 128), f32),
    pltpu.VMEM((256 * YR, 128), f32),
    pltpu.VMEM((4, 8, 128), f32),
    pltpu.VMEM((D, 128), f32),
]

@jax.jit
def pallas_concat_heads__sliding_block__ssm_conv_s4__prompt_kernel(A_x, A_wqkv, A_wo, B_u, B_A_re, B_A_im, B_B_re, B_B_im, B_C_re, B_C_im, B_log_dt, B_Dskip):
    out = pl.pallas_call(
        kernel,
        out_shape=jax.ShapeDtypeStruct((S, 2 * D), bf16),
        scratch_shapes=SCRATCH,
        compiler_params=pltpu.CompilerParams(vmem_limit_bytes=110 * 1024 * 1024),
        name="fused",
    )(A_x.reshape(S, D), A_wqkv, A_wo, B_u.reshape(S, D), B_A_re, B_A_im, B_B_re, B_B_im, B_C_re, B_C_im,
      B_log_dt.reshape(4, 128), B_Dskip.reshape(4, 128))
    return out.reshape(1, S, 2 * D)
```

```python
import functools
import math

import jax
import jax.numpy as jnp
from jax import lax
from jax.experimental import pallas as pl
from jax.experimental.pallas import tpu as pltpu

f32, bf16, i32 = jnp.float32, jnp.bfloat16, jnp.int32
S, D = 2048, 512
QSCALE = 0.25 * math.log2(math.e)
NEG = -1e30
T = 64
NC = S // T
PR = 33
YR = 40
SR = 9
NG = 32
GP = 8
LAG_R, LAG_C1, LAG_C2 = 4, 8, 12
NT = (((1,), (1,)), ((), ()))


def iota(shape, dim):
    return lax.broadcasted_iota(jnp.int32, shape, dim)


def pack(x):
    return pltpu.bitcast(x, i32)


def unpack(x):
    return pltpu.bitcast(x, bf16)


def mo(x, m):
    return x if isinstance(x, int) else pl.multiple_of(x, m)


def cmul(ar, ai, br, bi):
    return ar * br - ai * bi, ar * bi + ai * br


def vmax_tree(xs, ways=4):
    acc = [None] * ways
    for r, x in enumerate(xs):
        acc[r % ways] = x if acc[r % ways] is None else jnp.maximum(acc[r % ways], x)
    return functools.reduce(jnp.maximum, [a for a in acc if a is not None])


def repack_w(wqkv_ref, wp_s, n):
    wp_s[n] = pack(wqkv_ref[:, pl.ds(n * 128, 128)])


def repack_x(i, x_ref, xp_s):
    for kt in range(4):
        xp_s[kt] = pack(x_ref[pl.ds(mo(i * 256, 256), 256), pl.ds(kt * 128, 128)])


def proj_items(i, xp_s, wp_s, qc_s, k_s, vt_s):
    def mm(n):
        acc = None
        for kt in range(4):
            d = jnp.dot(unpack(xp_s[kt]), unpack(wp_s[n, pl.ds(kt * 64, 64), :]), preferred_element_type=f32)
            acc = d if acc is None else acc + d
        return acc

    def q_tile(hg):
        q = mm(hg) * QSCALE
        oddh = ((iota((64, 128), 1) // 16) % 2) == 1
        for j in range(2):
            a, b = q[j * 128:j * 128 + 64], q[j * 128 + 64:j * 128 + 128]
            m = jnp.concatenate([jnp.where(oddh, b, a), jnp.where(oddh, a, b)], 0).astype(bf16)
            qc_s[2 * i + j, pl.ds(hg * 64, 64), :] = pack(m.T)

    def k_tile(hg):
        k_s[hg, pl.ds(mo(i * 128, 128), 128), :] = pack(mm(4 + hg).astype(bf16))

    def v_tile(hg):
        v = mm(8 + hg)
        for j in range(2):
            vt_s[2 * i + j, pl.ds(hg * 64, 64), :] = pack(v[j * 128:(j + 1) * 128].astype(bf16).T)

    return [[functools.partial(f, hg) for f in (q_tile, k_tile, v_tile)] for hg in range(4)]


def win(qb, odd, static_edge):
    if static_edge:
        b = 2 * qb + (1 if odd else 0)
        rmin = max(0, 256 - 64 * b)
        return rmin, 64 * b - 256 + rmin
    return 0, qb * 128 - 256 + (64 if odd else 0)


def qk_stage(qb, gi, static_edge, qc_s, k_s, st, hooks=None):
    hg = gi // 2
    lo = iota((8, 128), 1) < 64
    zero = jnp.zeros((8, 128), i32)
    for hp in (2 * gi, 2 * gi + 1):
        t = 2 * (hp % 2)
        h1, h2 = 2 * hp, 2 * hp + 1
        q1 = qc_s[qb, pl.ds(h1 * 8, 8), :]
        q2 = qc_s[qb, pl.ds(h2 * 8, 8), :]
        for odd in (False, True):
            blocks = [zero] * 8
            blocks[h1 % 8] = jnp.where(lo, zero, q1) if odd else jnp.where(lo, q1, zero)
            blocks[h2 % 8] = jnp.where(lo, q2, zero) if odd else jnp.where(lo, zero, q2)
            w = unpack(jnp.concatenate(blocks, 0))
            rmin, key0 = win(qb, odd, static_edge)
            n = 320 - rmin
            kk = k_s[hg, pl.ds(mo(key0 // 2, 32), n // 2), :]
            sc = jnp.dot(unpack(kk), w, preferred_element_type=f32)
            st[t, pl.ds(rmin, n), :] = sc
            m0 = max(rmin, 64)
            if m0 < 256:
                mid = sc[m0 - rmin:256 - rmin]
                st[t, 320:328, :] = vmax_tree([mid[8 * r:8 * r + 8] for r in range((256 - m0) // 8)])
            if hooks:
                r_ = min(16, n // 16)
                for fn in hooks[t]:
                    fn(sc[8 * r_:8 * r_ + 8])
            t += 1


def smpv_stage(qb, gi, static_edge, st, vt_s, ot_s):
    mask = iota((64, 128), 0) > (iota((64, 128), 1) % 64)
    zero = jnp.zeros((64, 128), f32)
    take_e = (iota((32, 128), 1) < 64) == (iota((32, 128), 0) < 16)
    for hp in (2 * gi, 2 * gi + 1):
        t = 2 * (hp % 2)
        zs = []
        for odd in (False, True):
            rmin, _ = win(qb, odd, static_edge)
            has_top = rmin == 0
            m0 = max(rmin, 64)
            bot = st[t, 256:320, :]
            comb = jnp.where(mask, st[t, 0:64, :], bot) if has_top else jnp.where(mask, NEG, bot)
            mx = vmax_tree([comb[8 * r:8 * r + 8] for r in range(8)], 2)
            if m0 < 256:
                mx = jnp.maximum(mx, st[t, 320:328, :])
            m = jnp.max(mx, axis=0, keepdims=True)
            lacc = [None, None]

            def accum(p):
                for r in range(8):
                    v = p[8 * r:8 * r + 8]
                    lacc[r % 2] = v if lacc[r % 2] is None else lacc[r % 2] + v
                return p

            pc = accum(jnp.exp2(comb - m))
            pbot = jnp.where(mask, 0.0, pc)
            ptop = jnp.where(mask, pc, 0.0) if has_top else None

            def piece(k):
                if k < 0:
                    return None
                if k == 4:
                    return pbot
                if k == 0:
                    return ptop
                return accum(jnp.exp2(st[t, 64 * k:64 * k + 64, :] - m)) if k >= m0 // 64 else None

            sl = [(-1, 0), (1, 2), (3, 4)] if odd else [(0, 1), (2, 3), (4, -1)]
            z = None
            for ci in range(3):
                a, b = piece(sl[ci][0]), piece(sl[ci][1])
                if a is None and b is None:
                    continue
                ch = jnp.concatenate([zero if a is None else a, zero if b is None else b], 0).astype(bf16)
                vt = unpack(vt_s[qb - 2 + ci, pl.ds(hp * 16, 16), :])
                d = jnp.dot(vt, ch, preferred_element_type=f32)
                z = d if z is None else z + d
            l = jnp.sum(lacc[0] + lacc[1], axis=0, keepdims=True)
            zs.append(z * (1.0 / l))
            t += 1
        o = jnp.where(take_e, zs[0], zs[1]).astype(bf16)
        ot_s[qb, pl.ds(hp * 16, 16), :] = pack(o)


def oproj_tr(qb, ot_s, o_s):
    oddh = ((iota((32, 128), 1) // 16) % 2) == 1
    for g in range(4):
        tp = pack(unpack(ot_s[qb, pl.ds(g * 64, 64), :]).T)
        a, b = tp[0:32], tp[32:64]
        o_s[g] = jnp.concatenate([jnp.where(oddh, b, a), jnp.where(oddh, a, b)], 0)


def oproj_mm(qb, n, o_s, wo_ref, out_ref):
    acc = None
    for g in range(4):
        d = jnp.dot(unpack(o_s[g]), wo_ref[pl.ds(g * 128, 128), pl.ds(n * 128, 128)], preferred_element_type=f32)
        acc = d if acc is None else acc + d
    out_ref[pl.ds(mo(qb * 128, 128), 128), pl.ds(n * 128, 128)] = acc.astype(bf16)


def b_prep(blk, dtc_s, are, aim, bre, bim, cre, cim, base_s, l8_s, lt_s, rt_s, wre_s):
    r0 = mo(blk * 32, 32)
    rows = pl.ds(r0, 32)
    dtc = dtc_s[rows, :]
    zr = dtc * are[rows, :].astype(f32)
    zi = dtc * aim[rows, :].astype(f32)
    mag = jnp.exp(zr)
    lr, li = mag * jnp.cos(zi), mag * jnp.sin(zi)
    wr, wi = cmul(cre[rows, :].astype(f32), cim[rows, :].astype(f32),
                  dtc * bre[rows, :].astype(f32), dtc * bim[rows, :].astype(f32))
    wre_s[rows, :] = wr
    a, b = cmul(wr, wi, lr, li)
    m = jnp.sqrt(a * a + b * b)
    t = jnp.sqrt(0.5 * (m + jnp.abs(a)))
    ts = jnp.where(t > 0.0, t, 1.0)
    o = jnp.where(t > 0.0, 0.5 * b / ts, 0.0)
    pos = a >= 0.0
    rr = jnp.where(pos, t, jnp.abs(o))
    ri = jnp.where(pos, o, jnp.where(b >= 0.0, t, -t))
    rt_s[0, rows, :] = rr
    rt_s[1, rows, :] = ri
    pr, pi = rr, ri
    for s in range(8):
        base_s[0, pl.ds(r0 * 8 + s, 32, stride=8), :] = pr
        base_s[1, pl.ds(r0 * 8 + s, 32, stride=8), :] = pi
        if s < 7:
            pr, pi = cmul(pr, pi, lr, li)
    qr, qi = lr, li
    for k in range(6):
        qr, qi = qr * qr - qi * qi, 2.0 * qr * qi
        if k == 2:
            l8_s[0, rows, :] = qr
            l8_s[1, rows, :] = qi
    lt_s[0, rows, :] = qr
    lt_s[1, rows, :] = qi


def u_prep(q, u_ref, ur_s):
    tp, c = q // NC, q % NC
    r0 = mo(c * T, T)
    rev = 7 - iota((8, 128), 0)
    parts = []
    for j in range(2):
        v = u_ref[pl.ds(r0, T), pl.ds((2 * tp + j) * 128, 128)].astype(f32)
        parts += [jnp.take_along_axis(v[8 * (7 - k):8 * (8 - k), :], rev, axis=0) for k in range(8)]
    ur_s[pl.ds(tp * 128 * PR + c, 128, stride=PR), :] = jnp.concatenate(parts, axis=0).T


def gen_p(d, base_s, l8_s):
    r8 = mo(d * 8, 8)
    pr, pi = base_s[0, pl.ds(r8, 8), :], base_s[1, pl.ds(r8, 8), :]
    mr = jnp.broadcast_to(l8_s[0, pl.ds(d, 1), :], (8, 128))
    mi = jnp.broadcast_to(l8_s[1, pl.ds(d, 1), :], (8, 128))
    rs, is_ = [pr], [pi]
    for _ in range(7):
        pr, pi = cmul(pr, pi, mr, mi)
        rs.append(pr)
        is_.append(pi)
    return jnp.concatenate(rs, 0), jnp.concatenate(is_, 0)


def chan0(g):
    return (g // 16) * 256 + (g % 16) * 8


def b_gen(g, i, base_s, l8_s, psv, rel):
    d0 = chan0(g)
    w = [gen_p(d0 + i + 128 * j, base_s, l8_s) for j in range(2)]
    psv[rel, 0] = jnp.concatenate([w[0][0], w[1][0]], 0).astype(bf16)
    psv[rel, 1] = jnp.concatenate([w[0][1], w[1][1]], 0).astype(bf16)


def b_a2(g, i, ps_all, ur_s, sb):
    ps = ps_all.at[g * 8 + i]
    lo = iota((NC, 128), 1) < T
    x = ur_s[pl.ds((g * 8 + i) * PR, NC), :]
    lhs = jnp.concatenate([jnp.where(lo, x, 0.0), jnp.where(lo, 0.0, x)], 0).astype(bf16)
    sre = jnp.dot(lhs, ps[0], preferred_element_type=f32)
    sim = jnp.dot(lhs, ps[1], preferred_element_type=f32)
    for j in range(2):
        sb[j, 0, pl.ds(i, NC, stride=SR), :] = sre[j * NC:(j + 1) * NC]
        sb[j, 1, pl.ds(i, NC, stride=SR), :] = sim[j * NC:(j + 1) * NC]


def b_rec(g, c0, c1, lt_s, rt_s, sb, hs):
    d0 = chan0(g)
    for j in range(2):
        rows = pl.ds(mo(d0 + 128 * j, 8), 8)
        ar, ai = lt_s[0, rows, :], lt_s[1, rows, :]
        if c0 == 0:
            hr = sb[j, 0, pl.ds(0, 8), :]
            hi = -sb[j, 1, pl.ds(0, 8), :]
            sb[j, 0, pl.ds(0, 8), :] = rt_s[0, rows, :]
            sb[j, 1, pl.ds(0, 8), :] = -rt_s[1, rows, :]
        else:
            hr, hi = hs[j, 0], hs[j, 1]
        for c in range(max(c0, 1), c1):
            if c < NC - 1:
                sr = sb[j, 0, pl.ds(c * SR, 8), :]
                si = sb[j, 1, pl.ds(c * SR, 8), :]
            sb[j, 0, pl.ds(c * SR, 8), :] = hr
            sb[j, 1, pl.ds(c * SR, 8), :] = hi
            if c < NC - 1:
                hr, hi = ar * hr + ai * hi + sr, ar * hi - ai * hr - si
        if c1 < NC:
            hs[j, 0] = hr
            hs[j, 1] = hi


def b_c1(g, i, ps_all, sb, kc, yb_s):
    ps = ps_all.at[g * 8 + i]
    lo = iota((NC, 128), 1) < T
    row0 = iota((NC, 128), 0) == 0
    gre = jnp.concatenate([sb[j, 0, pl.ds(i, NC, stride=SR), :] for j in range(2)], 0).astype(bf16)
    gim = jnp.concatenate([sb[j, 1, pl.ds(i, NC, stride=SR), :] for j in range(2)], 0).astype(bf16)
    y = (lax.dot_general(gre, ps[0], NT, preferred_element_type=f32)
         + lax.dot_general(gim, ps[1], NT, preferred_element_type=f32))
    yi = jnp.where(lo, y[0:NC], y[NC:2 * NC])
    kc[pl.ds(i, 1), :] = yi[0:1, :]
    yb_s[pl.ds((g * 8 + i) * YR, NC), :] = jnp.where(row0, 0.0, yi)


def b_c2(g, i, ur_s, kc, yb_s):
    lane = iota((8, 128), 1)
    rev = 7 - iota((8, 128), 0)
    kcb = jnp.broadcast_to(kc[pl.ds(i, 1), :], (8, 128))
    h0, h1 = [], []
    for v in range(8):
        r = pltpu.roll(kcb, 57 - 8 * v, 1, stride=1, stride_axis=0)
        r = jnp.take_along_axis(r, rev, axis=0)
        sg = lane + iota((8, 128), 0) + 8 * v
        h0.append(jnp.where((lane < 64) & (sg >= 64), r, 0.0))
        h1.append(jnp.where(sg >= 128, r, 0.0))
    hk = jnp.concatenate(h0 + h1, 0).astype(bf16)
    x = ur_s[pl.ds((g * 8 + i) * PR, NC), :]
    rows = pl.ds((g * 8 + i) * YR, NC)
    yb_s[rows, :] = yb_s[rows, :] + jnp.dot(x.astype(bf16), hk, preferred_element_type=f32)


def b_out(q, u_ref, yb_s, coef_s, out_ref):
    tp, c = q // NC, q % NC
    mt = yb_s[pl.ds(tp * 128 * YR + c, 128, stride=YR), :].T
    r0 = mo(c * T, T)
    for j in range(2):
        lt = 2 * tp + j
        cf = coef_s[lt]
        uu = u_ref[pl.ds(r0, T), pl.ds(mo(lt * 128, 128), 128)].astype(f32)
        y = mt[j * T:(j + 1) * T] + uu * jnp.concatenate([cf] * 8, 0)
        out_ref[pl.ds(r0, T), pl.ds(mo(D + lt * 128, 128), 128)] = y.astype(bf16)


def kernel(x_hbm, wqkv_hbm, wo_hbm, u_hbm, are_h, aim_h, bre_h, bim_h, cre_h, cim_h, ldt_h, dsk_h, out_hbm,
           x_ref, wqkv_ref, wo_ref, u_ref, are, aim, bre, bim, cre, cim, ldt_ref, dsk_ref, out_ref,
           sem_p, sem_w, sem_x, sem_u, sem_o,
           wp_s, xp_s, qc_s, k_s, vt_s, ot_s, o_s, st0, st1,
           ur_s, base_s, l8_s, lt_s, rt_s, wre_s, sb0, sb1, sb2, sb3, ps_all, kc0, kc1, kc2, kc3, hs,
           yb_s, coef_s, dtc_s):
    def cp_x(i):
        rows = pl.ds(mo(i * 128, 128), 128)
        return pltpu.make_async_copy(x_hbm.at[rows, :], x_ref.at[rows, :], sem_x.at[i])

    def cp_u(i):
        sl = (pl.ds(mo((i % 4) * 512, 512), 512), pl.ds(mo((i // 4) * 256, 256), 256))
        return pltpu.make_async_copy(u_hbm.at[sl], u_ref.at[sl], sem_u.at[i])

    six = [(are_h, are), (aim_h, aim), (bre_h, bre), (bim_h, bim), (cre_h, cre), (cim_h, cim)]

    def rows_cp(r0, nr, k0):
        return [pltpu.make_async_copy(a.at[pl.ds(r0, nr), :], b.at[pl.ds(r0, nr), :], sem_p.at[k0 + n])
                for n, (a, b) in enumerate(six)]

    def cp_outA(qb):
        sl = (pl.ds(mo(qb * 128, 128), 128), pl.ds(0, D))
        return pltpu.make_async_copy(out_ref.at[sl], out_hbm.at[sl], sem_o.at[0])

    def cp_outB(qb):
        sl = (pl.ds(mo((qb % 4) * 512, 512), 512), pl.ds(mo(D + ((qb - 8) // 4) * 256, 256), 256))
        return pltpu.make_async_copy(out_ref.at[sl], out_hbm.at[sl], sem_o.at[1])

    small = [pltpu.make_async_copy(ldt_h, ldt_ref, sem_p.at[0]), pltpu.make_async_copy(dsk_h, dsk_ref, sem_p.at[1])]
    cp_par = rows_cp(0, 160, 2)
    cp_par2 = rows_cp(160, D - 160, 8)
    cp_w = [pltpu.make_async_copy(wqkv_hbm.at[:, pl.ds(512 * p, 512)], wqkv_ref.at[:, pl.ds(512 * p, 512)],
                                  sem_w.at[p]) for p in range(3)]
    cp_wo = pltpu.make_async_copy(wo_hbm, wo_ref, sem_w.at[3])
    LOW = dict(priority=1)

    for c in small:
        c.start()
    cp_x(0).start()
    cp_x(1).start()
    for c in cp_w:
        c.start()
    for c in cp_par:
        c.start(**LOW)
    cp_x(2).start(**LOW)
    cp_x(3).start(**LOW)
    cp_u(0).start(**LOW)
    cp_x(4).start(**LOW)
    cp_x(5).start(**LOW)

    sb = [sb0, sb1, sb2, sb3]
    kc = [kc0, kc1, kc2, kc3]
    st = [st0, st1]

    def prep_items(i):
        a = i + 4 * (i // 4)
        bg = []
        for k in range(2):
            bg.append(functools.partial(b_prep, a + 4 * k, dtc_s, are, aim, bre, bim, cre, cim,
                                        base_s, l8_s, lt_s, rt_s, wre_s))
            for k2 in range(4):
                bg.append(functools.partial(u_prep, i * 8 + k * 4 + k2, u_ref, ur_s))
        return bg

    for d in (0, 128):
        base_s[:, pl.ds(d * 8, GP * 8), :] = jnp.zeros((2, GP * 8, 128), f32)
        l8_s[:, pl.ds(d, GP), :] = jnp.zeros((2, GP, 128), f32)

    for c in small:
        c.wait()
    for g in range(4):
        dt = jnp.exp(ldt_ref[g:g + 1, :].astype(f32)).astype(bf16).astype(f32)
        dtc_s[g * 128:(g + 1) * 128, :] = jnp.broadcast_to(dt, (128, 128)).T
    cp_x(0).wait()
    cp_x(1).wait()
    repack_x(0, x_ref, xp_s)
    items = proj_items(0, xp_s, wp_s, qc_s, k_s, vt_s)
    for p in range(3):
        cp_w[p].wait()
        if p == 1:
            for c in cp_par2:
                c.start(**LOW)
            cp_u(1).start(**LOW)
        for hg in range(4):
            repack_w(wqkv_ref, wp_s, 4 * p + hg)
            items[hg][p]()
    for i_ in range(3, 8):
        cp_x(2 * i_).start(**LOW)
        cp_x(2 * i_ + 1).start(**LOW)
        cp_u(i_ - 1).start(**LOW)
    cp_u(7).start(**LOW)
    cp_wo.start(**LOW)
    for c in cp_par:
        c.wait()

    def phase1(i, c):
        @pl.when(i < 7)
        def _():
            cp_x(2 * i + 2).wait()
            cp_x(2 * i + 3).wait()
        cp_u(i - 1).wait()

        @pl.when(i == 2)
        def _():
            for c_ in cp_par2:
                c_.wait()
        its = proj_items(i, xp_s, wp_s, qc_s, k_s, vt_s)
        its = [its[hg][p] for hg in range(4) for p in (0, 2, 1)]
        qg = jnp.maximum(i - 2, 0)
        psv = ps_all.at[pl.ds(mo(qg * 32, 32), 32)]
        bg = [functools.partial(b_gen, qg * 4 + k // 8, k % 8, base_s, l8_s, psv, k) for k in range(GP)]
        bg = bg + prep_items(i - 1)
        n = len(its)
        for j in range(n):
            its[j]()
            for fn in bg[j * len(bg) // n:(j + 1) * len(bg) // n]:
                fn()
        repack_x(jnp.minimum(i + 1, 7), x_ref, xp_s)
        return c + (i >> 10)

    cp_x(2).wait()
    cp_x(3).wait()
    repack_x(1, x_ref, xp_s)
    zero_dyn = lax.fori_loop(1, 8, phase1, 0)
    cp_u(7).wait()
    cp_wo.wait()

    def body(qb, edge, next_edge, gen, bout, first=False):
        static = isinstance(qb, int)
        bg = [[] for _ in range(8)]
        if gen:
            qg = qb + 6 if static else qb - 2
            psv = ps_all.at[pl.ds(mo(qg * 32, 32), 32)]
        if not first:
            bg[0].append(functools.partial(oproj_tr, qb - 1, ot_s, o_s))
            for n in range(4):
                bg[4 + n].append(functools.partial(oproj_mm, qb - 1, n, o_s, wo_ref, out_ref))
        if bout:
            for k in range(8):
                bg[k].append(functools.partial(b_out, (qb - 8) * 8 + k, u_ref, yb_s, coef_s, out_ref))
        if first:
            its = prep_items(7)
            for n_, fn in enumerate(its):
                bg[n_ * 8 // len(its)].append(fn)
        for u in range(8):
            hooks = [[] for _ in range(4)]
            if gen:
                def gate(v, row=D * 8 + (zero_dyn if static else (qb >> 10))):
                    base_s[0, pl.ds(mo(row, 8), 8), :] = v
                ks = list(range(0 if static else GP, 32))
                ks = ks[u * len(ks) // 8:(u + 1) * len(ks) // 8]
                for n_, k in enumerate(ks):
                    t_ = 2 * (n_ * 2 // len(ks)) + 1
                    if not hooks[t_]:
                        hooks[t_].append(gate)
                    hooks[t_].append(lambda v, k=k: b_gen(qg * 4 + k // 8, k % 8, base_s, l8_s, psv, k))
            if u < 7:
                qk_stage(qb, u + 1, edge, qc_s, k_s, st[(u + 1) % 2], hooks)
            else:
                qn = qb + 1 if static else jnp.minimum(qb + 1, 15)
                qk_stage(qn, 0, next_edge, qc_s, k_s, st[(u + 1) % 2], hooks)
            for fn in bg[u]:
                fn()
            smpv_stage(qb, u, edge, st[u % 2], vt_s, ot_s)
        if not first:
            cp_outA(qb - 1).start()
        if bout:
            cp_outB(qb).start()

    qk_stage(0, 0, True, qc_s, k_s, st0)
    body(0, True, True, True, False, first=True)
    body(1, True, False, True, False)

    def loop_x(i, c):
        for r_ in range(2):
            body(2 + i * 2 + r_, False, False, True, False)
        return c
    lax.fori_loop(0, 3, loop_x, 0)

    ones = jnp.ones((8, 128), f32)
    for g in range(4):
        k0 = lax.dot_general(ones, wre_s[g * 128:(g + 1) * 128, :], NT, preferred_element_type=f32,
                             precision=lax.Precision.HIGHEST)
        coef_s[g] = k0 + jnp.broadcast_to(dsk_ref[g:g + 1, :].astype(f32), (8, 128))

    nslot = NG * 4
    for s0 in range(0, nslot + LAG_C2, 4):
        def live(lag):
            return [(s // 4, (s // 4) % 4, s % 4) for s in range(s0 - lag, s0 - lag + 4) if 0 <= s < nslot]
        for g, r, k in live(LAG_C1):
            for i in (2 * k, 2 * k + 1):
                b_c1(g, i, ps_all, sb[r], kc[r], yb_s)
        for g, r, k in live(LAG_C2):
            for i in (2 * k, 2 * k + 1):
                b_c2(g, i, ur_s, kc[r], yb_s)
        for g, r, k in live(0):
            for i in (2 * k, 2 * k + 1):
                b_a2(g, i, ps_all, ur_s, sb[r])
        for g, r, k in live(LAG_R):
            b_rec(g, 8 * k, 8 * k + 8, lt_s, rt_s, sb[r], hs)

    def loop_y(i, c):
        for r_ in range(2):
            body(8 + i * 2 + r_, False, False, False, True)
        return c
    lax.fori_loop(0, 4, loop_y, 0)

    oproj_tr(15, ot_s, o_s)
    for n in range(4):
        oproj_mm(15, n, o_s, wo_ref, out_ref)
    cp_outA(15).start()
    for qb in range(16):
        cp_outA(qb).wait()
    for qb in range(8, 16):
        cp_outB(qb).wait()


def _scratch():
    vm = pltpu.VMEM
    dma = pltpu.SemaphoreType.DMA
    return [
        vm((S, D), bf16), vm((D, 3 * D), bf16), vm((D, D), bf16), vm((S, D), bf16),
        *[vm((D, 128), bf16) for _ in range(6)], vm((4, 128), bf16), vm((4, 128), bf16),
        vm((S, 2 * D), bf16),
        dma((14,)), dma((4,)), dma((16,)), dma((8,)), dma((2,)),
        vm((12, 256, 128), i32),
        vm((4, 128, 128), i32),
        vm((16, 256, 128), i32),
        vm((4, S // 2, 128), i32),
        vm((16, 256, 128), i32),
        vm((16, 256, 128), i32),
        vm((4, 64, 128), i32),
        vm((4, 328, 128), f32), vm((4, 328, 128), f32),
        vm((256 * PR, 128), f32),
        vm((2, D * 8 + 8, 128), f32),
        vm((2, D, 128), f32), vm((2, D, 128), f32), vm((2, D, 128), f32),
        vm((D, 128), f32),
        *[vm((2, 2, NC * SR, 128), f32) for _ in range(4)],
        vm((256, 2, 128, 128), bf16),
        *[vm((8, 128), f32) for _ in range(4)],
        vm((2, 2, 8, 128), f32),
        vm((256 * YR, 128), f32),
        vm((4, 8, 128), f32),
        vm((D, 128), f32),
    ]


@jax.jit
def pallas_concat_heads__sliding_block__ssm_conv_s4__prompt_kernel(
    A_x: jax.Array,
    A_wqkv: jax.Array,
    A_wo: jax.Array,
    B_u: jax.Array,
    B_A_re: jax.Array,
    B_A_im: jax.Array,
    B_B_re: jax.Array,
    B_B_im: jax.Array,
    B_C_re: jax.Array,
    B_C_im: jax.Array,
    B_log_dt: jax.Array,
    B_Dskip: jax.Array,
):
    out = pl.pallas_call(
        kernel,
        out_shape=jax.ShapeDtypeStruct((S, 2 * D), bf16),
        in_specs=[pl.BlockSpec(memory_space=pl.ANY)] * 12,
        out_specs=pl.BlockSpec(memory_space=pl.ANY),
        scratch_shapes=_scratch(),
        compiler_params=pltpu.CompilerParams(
            vmem_limit_bytes=100 * 1024 * 1024,
            flags={"XLA_TPU_EVENLY_DISTRIBUTE_CRITICAL_NODES": True},
        ),
        name="fused",
    )(A_x.reshape(S, D), A_wqkv, A_wo, B_u.reshape(S, D), B_A_re, B_A_im, B_B_re, B_B_im, B_C_re, B_C_im,
      B_log_dt.reshape(4, 128), B_Dskip.reshape(4, 128))
    return out.reshape(1, S, 2 * D)
```

```python
import functools
import math

import jax
import jax.numpy as jnp
from jax import lax
from jax.experimental import pallas as pl
from jax.experimental.pallas import tpu as pltpu

f32, bf16, i32 = jnp.float32, jnp.bfloat16, jnp.int32
S, D = 2048, 512
QSCALE = 0.25 * math.log2(math.e)
NEG = -1e30
T = 64
NC = S // T
PR = 33
YR = 40
SR = 9
NG = 32
GP = 8
LAG_R, LAG_C1, LAG_C2 = 4, 8, 12
NT = (((1,), (1,)), ((), ()))


def iota(shape, dim):
    return lax.broadcasted_iota(jnp.int32, shape, dim)


def pack(x):
    return pltpu.bitcast(x, i32)


def unpack(x):
    return pltpu.bitcast(x, bf16)


def mo(x, m):
    return x if isinstance(x, int) else pl.multiple_of(x, m)


def cmul(ar, ai, br, bi):
    return ar * br - ai * bi, ar * bi + ai * br


def vmax_tree(xs, ways=4):
    acc = [None] * ways
    for r, x in enumerate(xs):
        acc[r % ways] = x if acc[r % ways] is None else jnp.maximum(acc[r % ways], x)
    return functools.reduce(jnp.maximum, [a for a in acc if a is not None])


def repack_w(wqkv_ref, wp_s, n):
    wp_s[n] = pack(wqkv_ref[:, pl.ds(n * 128, 128)])


def repack_x(i, x_ref, xp_s):
    for kt in range(4):
        xp_s[kt] = pack(x_ref[pl.ds(mo(i * 256, 256), 256), pl.ds(kt * 128, 128)])


def proj_items(i, xp_s, wp_s, qc_s, k_s, vt_s):
    def mm(n):
        acc = None
        for kt in range(4):
            d = jnp.dot(unpack(xp_s[kt]), unpack(wp_s[n, pl.ds(kt * 64, 64), :]), preferred_element_type=f32)
            acc = d if acc is None else acc + d
        return acc

    def q_tile(hg):
        q = mm(hg) * QSCALE
        oddh = ((iota((64, 128), 1) // 16) % 2) == 1
        for j in range(2):
            a, b = q[j * 128:j * 128 + 64], q[j * 128 + 64:j * 128 + 128]
            m = jnp.concatenate([jnp.where(oddh, b, a), jnp.where(oddh, a, b)], 0).astype(bf16)
            qc_s[2 * i + j, pl.ds(hg * 64, 64), :] = pack(m.T)

    def k_tile(hg):
        k_s[hg, pl.ds(mo(i * 128, 128), 128), :] = pack(mm(4 + hg).astype(bf16))

    def v_tile(hg):
        v = mm(8 + hg)
        for j in range(2):
            vt_s[2 * i + j, pl.ds(hg * 64, 64), :] = pack(v[j * 128:(j + 1) * 128].astype(bf16).T)

    return [[functools.partial(f, hg) for f in (q_tile, k_tile, v_tile)] for hg in range(4)]


def win(qb, odd, static_edge):
    if static_edge:
        b = 2 * qb + (1 if odd else 0)
        rmin = max(0, 256 - 64 * b)
        return rmin, 64 * b - 256 + rmin
    return 0, qb * 128 - 256 + (64 if odd else 0)


def qk_stage(qb, gi, static_edge, qc_s, k_s, st, hooks=None):
    hg = gi // 2
    lo = iota((8, 128), 1) < 64
    zero = jnp.zeros((8, 128), i32)
    for hp in (2 * gi, 2 * gi + 1):
        t = 2 * (hp % 2)
        h1, h2 = 2 * hp, 2 * hp + 1
        q1 = qc_s[qb, pl.ds(h1 * 8, 8), :]
        q2 = qc_s[qb, pl.ds(h2 * 8, 8), :]
        for odd in (False, True):
            blocks = [zero] * 8
            blocks[h1 % 8] = jnp.where(lo, zero, q1) if odd else jnp.where(lo, q1, zero)
            blocks[h2 % 8] = jnp.where(lo, q2, zero) if odd else jnp.where(lo, zero, q2)
            w = unpack(jnp.concatenate(blocks, 0))
            rmin, key0 = win(qb, odd, static_edge)
            n = 320 - rmin
            kk = k_s[hg, pl.ds(mo(key0 // 2, 32), n // 2), :]
            sc = jnp.dot(unpack(kk), w, preferred_element_type=f32)
            st[t, pl.ds(rmin, n), :] = sc
            m0 = max(rmin, 64)
            if m0 < 256:
                mid = sc[m0 - rmin:256 - rmin]
                st[t, 320:328, :] = vmax_tree([mid[8 * r:8 * r + 8] for r in range((256 - m0) // 8)])
            if hooks:
                r_ = min(16, n // 16)
                for fn in hooks[t]:
                    fn(sc[8 * r_:8 * r_ + 8])
            t += 1


def smpv_stage(qb, gi, static_edge, st, vt_s, ot_s):
    mask = iota((64, 128), 0) > (iota((64, 128), 1) % 64)
    zero = jnp.zeros((64, 128), f32)
    take_e = (iota((32, 128), 1) < 64) == (iota((32, 128), 0) < 16)
    for hp in (2 * gi, 2 * gi + 1):
        t = 2 * (hp % 2)
        zs = []
        for odd in (False, True):
            rmin, _ = win(qb, odd, static_edge)
            has_top = rmin == 0
            m0 = max(rmin, 64)
            bot = st[t, 256:320, :]
            comb = jnp.where(mask, st[t, 0:64, :], bot) if has_top else jnp.where(mask, NEG, bot)
            mx = vmax_tree([comb[8 * r:8 * r + 8] for r in range(8)], 2)
            if m0 < 256:
                mx = jnp.maximum(mx, st[t, 320:328, :])
            m = jnp.max(mx, axis=0, keepdims=True)
            lacc = [None, None]

            def accum(p):
                for r in range(8):
                    v = p[8 * r:8 * r + 8]
                    lacc[r % 2] = v if lacc[r % 2] is None else lacc[r % 2] + v
                return p

            pc = accum(jnp.exp2(comb - m))
            pbot = jnp.where(mask, 0.0, pc)
            ptop = jnp.where(mask, pc, 0.0) if has_top else None

            def piece(k):
                if k < 0:
                    return None
                if k == 4:
                    return pbot
                if k == 0:
                    return ptop
                return accum(jnp.exp2(st[t, 64 * k:64 * k + 64, :] - m)) if k >= m0 // 64 else None

            sl = [(-1, 0), (1, 2), (3, 4)] if odd else [(0, 1), (2, 3), (4, -1)]
            z = None
            for ci in range(3):
                a, b = piece(sl[ci][0]), piece(sl[ci][1])
                if a is None and b is None:
                    continue
                ch = jnp.concatenate([zero if a is None else a, zero if b is None else b], 0).astype(bf16)
                vt = unpack(vt_s[qb - 2 + ci, pl.ds(hp * 16, 16), :])
                d = jnp.dot(vt, ch, preferred_element_type=f32)
                z = d if z is None else z + d
            l = jnp.sum(lacc[0] + lacc[1], axis=0, keepdims=True)
            zs.append(z * (1.0 / l))
            t += 1
        o = jnp.where(take_e, zs[0], zs[1]).astype(bf16)
        ot_s[qb, pl.ds(hp * 16, 16), :] = pack(o)


def oproj_tr(qb, ot_s, o_s):
    oddh = ((iota((32, 128), 1) // 16) % 2) == 1
    for g in range(4):
        tp = pack(unpack(ot_s[qb, pl.ds(g * 64, 64), :]).T)
        a, b = tp[0:32], tp[32:64]
        o_s[g] = jnp.concatenate([jnp.where(oddh, b, a), jnp.where(oddh, a, b)], 0)


def oproj_mm(qb, n, o_s, wo_ref, out_ref):
    acc = None
    for g in range(4):
        d = jnp.dot(unpack(o_s[g]), wo_ref[pl.ds(g * 128, 128), pl.ds(n * 128, 128)], preferred_element_type=f32)
        acc = d if acc is None else acc + d
    out_ref[pl.ds(mo(qb * 128, 128), 128), pl.ds(n * 128, 128)] = acc.astype(bf16)


def b_prep(blk, dtc_s, are, aim, bre, bim, cre, cim, base_s, l8_s, lt_s, rt_s, wre_s):
    r0 = mo(blk * 32, 32)
    rows = pl.ds(r0, 32)
    dtc = dtc_s[rows, :]
    zr = dtc * are[rows, :].astype(f32)
    zi = dtc * aim[rows, :].astype(f32)
    mag = jnp.exp(zr)
    lr, li = mag * jnp.cos(zi), mag * jnp.sin(zi)
    wr, wi = cmul(cre[rows, :].astype(f32), cim[rows, :].astype(f32),
                  dtc * bre[rows, :].astype(f32), dtc * bim[rows, :].astype(f32))
    wre_s[rows, :] = wr
    a, b = cmul(wr, wi, lr, li)
    m = jnp.sqrt(a * a + b * b)
    t = jnp.sqrt(0.5 * (m + jnp.abs(a)))
    ts = jnp.where(t > 0.0, t, 1.0)
    o = jnp.where(t > 0.0, 0.5 * b / ts, 0.0)
    pos = a >= 0.0
    rr = jnp.where(pos, t, jnp.abs(o))
    ri = jnp.where(pos, o, jnp.where(b >= 0.0, t, -t))
    rt_s[0, rows, :] = rr
    rt_s[1, rows, :] = ri
    pr, pi = rr, ri
    for s in range(8):
        base_s[0, pl.ds(r0 * 8 + s, 32, stride=8), :] = pr
        base_s[1, pl.ds(r0 * 8 + s, 32, stride=8), :] = pi
        if s < 7:
            pr, pi = cmul(pr, pi, lr, li)
    qr, qi = lr, li
    for k in range(6):
        qr, qi = qr * qr - qi * qi, 2.0 * qr * qi
        if k == 2:
            l8_s[0, rows, :] = qr
            l8_s[1, rows, :] = qi
    lt_s[0, rows, :] = qr
    lt_s[1, rows, :] = qi


def u_prep(q, u_ref, ur_s):
    tp, c = q // NC, q % NC
    r0 = mo(c * T, T)
    rev = 7 - iota((8, 128), 0)
    parts = []
    for j in range(2):
        v = u_ref[pl.ds(r0, T), pl.ds((2 * tp + j) * 128, 128)].astype(f32)
        parts += [jnp.take_along_axis(v[8 * (7 - k):8 * (8 - k), :], rev, axis=0) for k in range(8)]
    ur_s[pl.ds(tp * 128 * PR + c, 128, stride=PR), :] = jnp.concatenate(parts, axis=0).T


def gen_p(d, base_s, l8_s):
    r8 = mo(d * 8, 8)
    pr, pi = base_s[0, pl.ds(r8, 8), :], base_s[1, pl.ds(r8, 8), :]
    mr = jnp.broadcast_to(l8_s[0, pl.ds(d, 1), :], (8, 128))
    mi = jnp.broadcast_to(l8_s[1, pl.ds(d, 1), :], (8, 128))
    rs, is_ = [pr], [pi]
    for _ in range(7):
        pr, pi = cmul(pr, pi, mr, mi)
        rs.append(pr)
        is_.append(pi)
    return jnp.concatenate(rs, 0), jnp.concatenate(is_, 0)


def chan0(g):
    return (g // 16) * 256 + (g % 16) * 8


def b_gen(g, i, base_s, l8_s, psv, rel):
    d0 = chan0(g)
    w = [gen_p(d0 + i + 128 * j, base_s, l8_s) for j in range(2)]
    psv[rel, 0] = jnp.concatenate([w[0][0], w[1][0]], 0).astype(bf16)
    psv[rel, 1] = jnp.concatenate([w[0][1], w[1][1]], 0).astype(bf16)


def b_a2(g, i, ps_all, ur_s, sb):
    ps = ps_all.at[g * 8 + i]
    lo = iota((NC, 128), 1) < T
    x = ur_s[pl.ds((g * 8 + i) * PR, NC), :]
    lhs = jnp.concatenate([jnp.where(lo, x, 0.0), jnp.where(lo, 0.0, x)], 0).astype(bf16)
    sre = jnp.dot(lhs, ps[0], preferred_element_type=f32)
    sim = jnp.dot(lhs, ps[1], preferred_element_type=f32)
    for j in range(2):
        sb[j, 0, pl.ds(i, NC, stride=SR), :] = sre[j * NC:(j + 1) * NC]
        sb[j, 1, pl.ds(i, NC, stride=SR), :] = sim[j * NC:(j + 1) * NC]


def b_rec(g, c0, c1, lt_s, rt_s, sb, hs):
    d0 = chan0(g)
    for j in range(2):
        rows = pl.ds(mo(d0 + 128 * j, 8), 8)
        ar, ai = lt_s[0, rows, :], lt_s[1, rows, :]
        if c0 == 0:
            hr = sb[j, 0, pl.ds(0, 8), :]
            hi = -sb[j, 1, pl.ds(0, 8), :]
            sb[j, 0, pl.ds(0, 8), :] = rt_s[0, rows, :]
            sb[j, 1, pl.ds(0, 8), :] = -rt_s[1, rows, :]
        else:
            hr, hi = hs[j, 0], hs[j, 1]
        for c in range(max(c0, 1), c1):
            if c < NC - 1:
                sr = sb[j, 0, pl.ds(c * SR, 8), :]
                si = sb[j, 1, pl.ds(c * SR, 8), :]
            sb[j, 0, pl.ds(c * SR, 8), :] = hr
            sb[j, 1, pl.ds(c * SR, 8), :] = hi
            if c < NC - 1:
                hr, hi = ar * hr + ai * hi + sr, ar * hi - ai * hr - si
        if c1 < NC:
            hs[j, 0] = hr
            hs[j, 1] = hi


def b_c1(g, i, ps_all, sb, kc, yb_s):
    ps = ps_all.at[g * 8 + i]
    lo = iota((NC, 128), 1) < T
    row0 = iota((NC, 128), 0) == 0
    gre = jnp.concatenate([sb[j, 0, pl.ds(i, NC, stride=SR), :] for j in range(2)], 0).astype(bf16)
    gim = jnp.concatenate([sb[j, 1, pl.ds(i, NC, stride=SR), :] for j in range(2)], 0).astype(bf16)
    y = (lax.dot_general(gre, ps[0], NT, preferred_element_type=f32)
         + lax.dot_general(gim, ps[1], NT, preferred_element_type=f32))
    yi = jnp.where(lo, y[0:NC], y[NC:2 * NC])
    kc[pl.ds(i, 1), :] = yi[0:1, :]
    yb_s[pl.ds((g * 8 + i) * YR, NC), :] = jnp.where(row0, 0.0, yi)


def b_c2(g, i, ur_s, kc, yb_s):
    lane = iota((8, 128), 1)
    rev = 7 - iota((8, 128), 0)
    kcb = jnp.broadcast_to(kc[pl.ds(i, 1), :], (8, 128))
    h0, h1 = [], []
    for v in range(8):
        r = pltpu.roll(kcb, 57 - 8 * v, 1, stride=1, stride_axis=0)
        r = jnp.take_along_axis(r, rev, axis=0)
        sg = lane + iota((8, 128), 0) + 8 * v
        h0.append(jnp.where((lane < 64) & (sg >= 64), r, 0.0))
        h1.append(jnp.where(sg >= 128, r, 0.0))
    hk = jnp.concatenate(h0 + h1, 0).astype(bf16)
    x = ur_s[pl.ds((g * 8 + i) * PR, NC), :]
    rows = pl.ds((g * 8 + i) * YR, NC)
    yb_s[rows, :] = yb_s[rows, :] + jnp.dot(x.astype(bf16), hk, preferred_element_type=f32)


def b_out(q, u_ref, yb_s, coef_s, out_ref):
    tp, c = q // NC, q % NC
    mt = yb_s[pl.ds(tp * 128 * YR + c, 128, stride=YR), :].T
    r0 = mo(c * T, T)
    for j in range(2):
        lt = 2 * tp + j
        cf = coef_s[lt]
        uu = u_ref[pl.ds(r0, T), pl.ds(mo(lt * 128, 128), 128)].astype(f32)
        y = mt[j * T:(j + 1) * T] + uu * jnp.concatenate([cf] * 8, 0)
        out_ref[pl.ds(r0, T), pl.ds(mo(D + lt * 128, 128), 128)] = y.astype(bf16)


def kernel(x_hbm, wqkv_hbm, wo_hbm, u_hbm, are_h, aim_h, bre_h, bim_h, cre_h, cim_h, ldt_h, dsk_h, out_hbm,
           x_ref, wqkv_ref, wo_ref, u_ref, are, aim, bre, bim, cre, cim, ldt_ref, dsk_ref, out_ref,
           sem_p, sem_w, sem_x, sem_u, sem_o,
           wp_s, xp_s, qc_s, k_s, vt_s, ot_s, o_s, st0, st1,
           ur_s, base_s, l8_s, lt_s, rt_s, wre_s, sb0, sb1, sb2, sb3, ps_all, kc0, kc1, kc2, kc3, hs,
           yb_s, coef_s, dtc_s):
    def cp_x(i):
        rows = pl.ds(mo(i * 128, 128), 128)
        return pltpu.make_async_copy(x_hbm.at[rows, :], x_ref.at[rows, :], sem_x.at[i])

    def cp_u(i):
        sl = (pl.ds(mo((i % 4) * 512, 512), 512), pl.ds(mo((i // 4) * 256, 256), 256))
        return pltpu.make_async_copy(u_hbm.at[sl], u_ref.at[sl], sem_u.at[i])

    six = [(are_h, are), (aim_h, aim), (bre_h, bre), (bim_h, bim), (cre_h, cre), (cim_h, cim)]

    def rows_cp(r0, nr, k0):
        return [pltpu.make_async_copy(a.at[pl.ds(r0, nr), :], b.at[pl.ds(r0, nr), :], sem_p.at[k0 + n])
                for n, (a, b) in enumerate(six)]

    def cp_outA(qb):
        sl = (pl.ds(mo(qb * 128, 128), 128), pl.ds(0, D))
        return pltpu.make_async_copy(out_ref.at[sl], out_hbm.at[sl], sem_o.at[0])

    def cp_outB(qb):
        sl = (pl.ds(mo((qb % 4) * 512, 512), 512), pl.ds(mo(D + ((qb - 8) // 4) * 256, 256), 256))
        return pltpu.make_async_copy(out_ref.at[sl], out_hbm.at[sl], sem_o.at[1])

    small = [pltpu.make_async_copy(ldt_h, ldt_ref, sem_p.at[0]), pltpu.make_async_copy(dsk_h, dsk_ref, sem_p.at[1])]
    cp_par = rows_cp(0, 192, 2)
    cp_par2 = rows_cp(192, D - 192, 8)
    cp_w = [pltpu.make_async_copy(wqkv_hbm.at[:, pl.ds(512 * p, 512)], wqkv_ref.at[:, pl.ds(512 * p, 512)],
                                  sem_w.at[p]) for p in range(3)]
    cp_wo = pltpu.make_async_copy(wo_hbm, wo_ref, sem_w.at[3])
    LOW = dict(priority=1)

    for c in small:
        c.start()
    cp_x(0).start()
    cp_x(1).start()
    cp_w[0].start()
    cp_w[1].start()
    for c in cp_par:
        c.start()
    cp_w[2].start()
    cp_x(2).start(**LOW)
    cp_x(3).start(**LOW)
    cp_u(0).start(**LOW)
    cp_x(4).start(**LOW)
    cp_x(5).start(**LOW)

    sb = [sb0, sb1, sb2, sb3]
    kc = [kc0, kc1, kc2, kc3]
    st = [st0, st1]

    def prep_items(i, iu):
        bg = []
        for k in range(2):
            if i is not None:
                bg.append(functools.partial(b_prep, i + 4 * (i // 4) + 4 * k, dtc_s, are, aim, bre, bim, cre, cim,
                                            base_s, l8_s, lt_s, rt_s, wre_s))
            if iu is not None:
                for k2 in range(4):
                    bg.append(functools.partial(u_prep, iu * 8 + k * 4 + k2, u_ref, ur_s))
        return bg

    for c in small:
        c.wait()
    for g in range(4):
        dt = jnp.exp(ldt_ref[g:g + 1, :].astype(f32)).astype(bf16).astype(f32)
        dtc_s[g * 128:(g + 1) * 128, :] = jnp.broadcast_to(dt, (128, 128)).T
    cp_x(0).wait()
    cp_x(1).wait()
    repack_x(0, x_ref, xp_s)
    items = proj_items(0, xp_s, wp_s, qc_s, k_s, vt_s)
    for p in range(3):
        cp_w[p].wait()
        if p == 1:
            for c in cp_par2:
                c.start(**LOW)
            cp_u(1).start(**LOW)
        pre = []
        if p == 2:
            for c in cp_par:
                c.wait()
            pre = prep_items(0, None)
        for hg in range(4):
            repack_w(wqkv_ref, wp_s, 4 * p + hg)
            items[hg][p]()
            if pre and hg % 2 == 0:
                pre[hg // 2]()
    for i_ in range(3, 8):
        cp_x(2 * i_).start(**LOW)
        cp_x(2 * i_ + 1).start(**LOW)
        cp_u(i_ - 1).start(**LOW)
    cp_u(7).start(**LOW)
    cp_wo.start(**LOW)

    def phase1(i, c):
        @pl.when(i < 7)
        def _():
            cp_x(2 * i + 2).wait()
            cp_x(2 * i + 3).wait()
        cp_u(i - 1).wait()

        @pl.when(i == 2)
        def _():
            for c_ in cp_par2:
                c_.wait()
        its = proj_items(i, xp_s, wp_s, qc_s, k_s, vt_s)
        its = [its[hg][p] for hg in range(4) for p in (0, 2, 1)]
        qg = i - 1
        psv = ps_all.at[pl.ds(mo(qg * 32, 32), 32)]
        bg = [functools.partial(b_gen, qg * 4 + k // 8, k % 8, base_s, l8_s, psv, k) for k in range(GP)]
        bg = bg + prep_items(i, i - 1)
        n = len(its)
        for j in range(n):
            its[j]()
            for fn in bg[j * len(bg) // n:(j + 1) * len(bg) // n]:
                fn()
        repack_x(jnp.minimum(i + 1, 7), x_ref, xp_s)
        return c + (i >> 10)

    cp_x(2).wait()
    cp_x(3).wait()
    repack_x(1, x_ref, xp_s)
    zero_dyn = lax.fori_loop(1, 8, phase1, 0)
    cp_u(7).wait()
    cp_wo.wait()

    def body(qb, edge, next_edge, gen, bout, first=False):
        static = isinstance(qb, int)
        bg = [[] for _ in range(8)]
        if gen:
            qg = qb + 6 if static else qb - 2
            psv = ps_all.at[pl.ds(mo(qg * 32, 32), 32)]
        if not first:
            bg[0].append(functools.partial(oproj_tr, qb - 1, ot_s, o_s))
            for n in range(4):
                bg[4 + n].append(functools.partial(oproj_mm, qb - 1, n, o_s, wo_ref, out_ref))
        if bout:
            for k in range(8):
                bg[k].append(functools.partial(b_out, (qb - 8) * 8 + k, u_ref, yb_s, coef_s, out_ref))
        if first:
            its = prep_items(None, 7)
            for n_, fn in enumerate(its):
                bg[n_ * 8 // len(its)].append(fn)
        for u in range(8):
            hooks = [[] for _ in range(4)]
            if gen:
                def gate(v, row=D * 8 + (zero_dyn if static else (qb >> 10))):
                    base_s[0, pl.ds(mo(row, 8), 8), :] = v
                ks = list(range(0 if static and qb == 1 else GP, 32))
                ks = ks[u * len(ks) // 8:(u + 1) * len(ks) // 8]
                for n_, k in enumerate(ks):
                    t_ = 2 * (n_ * 2 // len(ks)) + 1
                    if not hooks[t_]:
                        hooks[t_].append(gate)
                    hooks[t_].append(lambda v, k=k: b_gen(qg * 4 + k // 8, k % 8, base_s, l8_s, psv, k))
            if u < 7:
                qk_stage(qb, u + 1, edge, qc_s, k_s, st[(u + 1) % 2], hooks)
            else:
                qn = qb + 1 if static else jnp.minimum(qb + 1, 15)
                qk_stage(qn, 0, next_edge, qc_s, k_s, st[(u + 1) % 2], hooks)
            for fn in bg[u]:
                fn()
            smpv_stage(qb, u, edge, st[u % 2], vt_s, ot_s)
        if not first:
            cp_outA(qb - 1).start()
        if bout:
            cp_outB(qb).start()

    qk_stage(0, 0, True, qc_s, k_s, st0)
    body(0, True, True, True, False, first=True)
    body(1, True, False, True, False)

    def loop_x(i, c):
        for r_ in range(2):
            body(2 + i * 2 + r_, False, False, True, False)
        return c
    lax.fori_loop(0, 3, loop_x, 0)

    ones = jnp.ones((8, 128), f32)
    for g in range(4):
        k0 = lax.dot_general(ones, wre_s[g * 128:(g + 1) * 128, :], NT, preferred_element_type=f32,
                             precision=lax.Precision.HIGHEST)
        coef_s[g] = k0 + jnp.broadcast_to(dsk_ref[g:g + 1, :].astype(f32), (8, 128))

    nslot = NG * 4
    for s0 in range(0, nslot + LAG_C2, 4):
        def live(lag):
            return [(s // 4, (s // 4) % 4, s % 4) for s in range(s0 - lag, s0 - lag + 4) if 0 <= s < nslot]
        for g, r, k in live(LAG_C1):
            for i in (2 * k, 2 * k + 1):
                b_c1(g, i, ps_all, sb[r], kc[r], yb_s)
        for g, r, k in live(LAG_C2):
            for i in (2 * k, 2 * k + 1):
                b_c2(g, i, ur_s, kc[r], yb_s)
        for g, r, k in live(0):
            for i in (2 * k, 2 * k + 1):
                b_a2(g, i, ps_all, ur_s, sb[r])
        for g, r, k in live(LAG_R):
            b_rec(g, 8 * k, 8 * k + 8, lt_s, rt_s, sb[r], hs)

    def loop_y(i, c):
        for r_ in range(2):
            body(8 + i * 2 + r_, False, False, False, True)
        return c
    lax.fori_loop(0, 4, loop_y, 0)

    oproj_tr(15, ot_s, o_s)
    last = []
    for n in range(4):
        oproj_mm(15, n, o_s, wo_ref, out_ref)
        if n % 2 == 1:
            sl = (pl.ds(15 * 128, 128), pl.ds((n - 1) * 128, 256))
            last.append(pltpu.make_async_copy(out_ref.at[sl], out_hbm.at[sl], sem_o.at[0]))
            last[-1].start()
    for qb in range(15):
        cp_outA(qb).wait()
    for c in last:
        c.wait()
    for qb in range(8, 16):
        cp_outB(qb).wait()


def _scratch():
    vm = pltpu.VMEM
    dma = pltpu.SemaphoreType.DMA
    return [
        vm((S, D), bf16), vm((D, 3 * D), bf16), vm((D, D), bf16), vm((S, D), bf16),
        *[vm((D, 128), bf16) for _ in range(6)], vm((4, 128), bf16), vm((4, 128), bf16),
        vm((S, 2 * D), bf16),
        dma((14,)), dma((4,)), dma((16,)), dma((8,)), dma((2,)),
        vm((12, 256, 128), i32),
        vm((4, 128, 128), i32),
        vm((16, 256, 128), i32),
        vm((4, S // 2, 128), i32),
        vm((16, 256, 128), i32),
        vm((16, 256, 128), i32),
        vm((4, 64, 128), i32),
        vm((4, 328, 128), f32), vm((4, 328, 128), f32),
        vm((256 * PR + 40, 128), f32),
        vm((2, D * 8 + 8, 128), f32),
        vm((2, D, 128), f32), vm((2, D, 128), f32), vm((2, D, 128), f32),
        vm((D, 128), f32),
        *[vm((2, 2, NC * SR + 8, 128), f32) for _ in range(4)],
        vm((256, 2, 128, 128), bf16),
        *[vm((8, 128), f32) for _ in range(4)],
        vm((2, 2, 8, 128), f32),
        vm((256 * YR + 40, 128), f32),
        vm((4, 8, 128), f32),
        vm((D, 128), f32),
    ]


@jax.jit
def pallas_concat_heads__sliding_block__ssm_conv_s4__prompt_kernel(
    A_x: jax.Array,
    A_wqkv: jax.Array,
    A_wo: jax.Array,
    B_u: jax.Array,
    B_A_re: jax.Array,
    B_A_im: jax.Array,
    B_B_re: jax.Array,
    B_B_im: jax.Array,
    B_C_re: jax.Array,
    B_C_im: jax.Array,
    B_log_dt: jax.Array,
    B_Dskip: jax.Array,
):
    out = pl.pallas_call(
        kernel,
        out_shape=jax.ShapeDtypeStruct((S, 2 * D), bf16),
        in_specs=[pl.BlockSpec(memory_space=pl.ANY)] * 12,
        out_specs=pl.BlockSpec(memory_space=pl.ANY),
        scratch_shapes=_scratch(),
        compiler_params=pltpu.CompilerParams(
            vmem_limit_bytes=100 * 1024 * 1024,
            flags={"XLA_TPU_EVENLY_DISTRIBUTE_CRITICAL_NODES": True},
        ),
        name="fused",
    )(A_x.reshape(S, D), A_wqkv, A_wo, B_u.reshape(S, D), B_A_re, B_A_im, B_B_re, B_B_im, B_C_re, B_C_im,
      B_log_dt.reshape(4, 128), B_Dskip.reshape(4, 128))
    return out.reshape(1, S, 2 * D)
```
